```python
import os as _os
_os.environ.setdefault("JAX_PLATFORMS", "cpu")
import jax
import jax.numpy as jnp

def _softmax(x, axis=-1):
    return jax.nn.softmax(x, axis=axis)
def _gelu(x):
    return jax.nn.gelu(x, approximate=True)
def _silu(x):
    return jax.nn.silu(x)
def _sigmoid(x):
    return jax.nn.sigmoid(x)
def _layernorm(x, axis=-1, eps=1e-5):
    m = jnp.mean(x, axis=axis, keepdims=True)
    v = jnp.var(x, axis=axis, keepdims=True)
    return (x - m) / jnp.sqrt(v + eps)
def _scatter_add(tgt, idx, src, axis=0):
    return tgt.at[idx].add(src)
def _segment_sum(src, seg, n):
    return jax.ops.segment_sum(src, seg, n)
class _Rng:
    def __init__(self, key):
        self._k = key
    def _next(self):
        self._k, sub = jax.random.split(self._k)
        return sub
    def normal(self, shape):
        return jax.random.normal(self._next(), shape, dtype=jnp.bfloat16)
    def randint(self, lo, hi, shape):
        return jax.random.randint(self._next(), shape, lo, hi, dtype=jnp.int32)
    def uniform(self, shape, lo=0.0, hi=1.0):
        return jax.random.uniform(self._next(), shape, jnp.bfloat16, lo, hi)
    def permutation(self, n):
        return jax.random.permutation(self._next(), n)


kernel_name = 'recurrent_scan__grouped_kv_mqa__mixer_s_mlp__prompt'

def setup_inputs():
    _rng = _Rng(jax.random.key(int.from_bytes(__import__("os").urandom(4), "little")))
    _w = (lambda a: (lambda t: t.astype(jnp.bfloat16) if jnp.issubdtype(t.dtype, jnp.floating) else t)(jnp.asarray(a)))
    def _A_setup():
        B, S, D, H = 1, 2048, 512, 32
        Dh = D // H
        return {
            "x": _w((lambda *s: _rng.normal(s) * 0.05)(B, S, D)),
            "wq": _w((lambda *s: _rng.normal(s) * 0.05)(D, H * Dh)),
            "wk": _w((lambda *s: _rng.normal(s) * 0.05)(D, Dh)),
            "wv": _w((lambda *s: _rng.normal(s) * 0.05)(D, Dh)),
            "wo": _w((lambda *s: _rng.normal(s) * 0.05)(H * Dh, D)),
        }
    _A_in = _A_setup()

    def _B_setup():
        B, S, D, F = 1, 2048, 512, 1792
        return {
            "x":  _w((lambda *s: _rng.normal(s) * 0.05)(B, S, D)),
            "w1": _w((lambda *s: _rng.normal(s) * 0.8)(D, D) * (D ** -0.5)),
            "w2": _w((lambda *s: _rng.normal(s) * 0.8)(D, D) * (D ** -0.5)),
            "w3": _w((lambda *s: _rng.normal(s) * 0.8)(D, F) * (D ** -0.5)),
            "w4": _w((lambda *s: _rng.normal(s) * 0.8)(F, D) * (F ** -0.5)),
        }
    _B_in = _B_setup()

    return {
        "A_x": _A_in["x"],
        "A_wq": _A_in["wq"],
        "A_wk": _A_in["wk"],
        "A_wv": _A_in["wv"],
        "A_wo": _A_in["wo"],
        "B_x": _B_in["x"],
        "B_w1": _B_in["w1"],
        "B_w2": _B_in["w2"],
        "B_w3": _B_in["w3"],
        "B_w4": _B_in["w4"],
    }

def reference(A_x, A_wq, A_wk, A_wv, A_wo, B_x, B_w1, B_w2, B_w3, B_w4):
    def _A_ref(x, wq, wk, wv, wo):
        B, S, D = x.shape
        H = 32
        Dh = D // H
        q = (lambda x, *d: x.transpose(*d))((x @ wq).reshape(B, S, H, Dh), 0, 2, 1, 3)
        k = x @ wk
        v = x @ wv
        scores = jnp.einsum("bhqd,bkd->bhqk", q, k) * (Dh ** -0.5)
        p = _softmax(scores, axis=-1)
        o = jnp.einsum("bhqk,bkd->bhqd", p, v)
        return (lambda x, *d: x.transpose(*d))(o, 0, 2, 1, 3).reshape(B, S, H * Dh) @ wo

    def _B_ref(x, w1, w2, w3, w4):
        B, S, D = x.shape
        h = _gelu(_layernorm(x, axis=-1) @ w1)
        c = D // 4
        g0 = jnp.pad(h[:, :, 0*c:1*c], ((0, 0), (1, 0), (0, 0)))[:, :S, :]
        g1 = jnp.pad(h[:, :, 1*c:2*c], ((0, 0), (0, 1), (0, 0)))[:, 1:, :]
        g2 = jnp.pad(h[:, :, 2*c:3*c], ((0, 0), (2, 0), (0, 0)))[:, :S, :]
        g3 = jnp.pad(h[:, :, 3*c:   ], ((0, 0), (0, 2), (0, 0)))[:, 2:, :]
        hs = jnp.concatenate([g0, g1, g2, g3], axis=-1) @ w2
        x1 = x + hs
        h2 = _gelu(_layernorm(x1, axis=-1) @ w3) @ w4
        return x1 + h2

    x = A_x
    xn = _layernorm(x, axis=-1)
    s = _A_ref(xn, A_wq, A_wk, A_wv, A_wo)
    g = _silu(_B_ref(xn, B_w1, B_w2, B_w3, B_w4))
    return x + s * g
```

```python
import functools
import jax
import jax.numpy as jnp
from jax import lax
import jax.experimental.pallas as pl
import jax.experimental.pallas.tpu as pltpu

S, D, H, DH, F = 2048, 512, 32, 16, 1792
F32, BF16 = jnp.float32, jnp.bfloat16
LOG2E = 1.4426950408889634
PADR = 16

def _ln(x):
    m = jnp.mean(x, axis=-1, keepdims=True)
    xc = x - m
    v = jnp.mean(xc * xc, axis=-1, keepdims=True)
    return xc * lax.rsqrt(v + 1e-5)

def _gelu(x):
    c = 0.7978845608028654
    return (0.5 * x) * (1.0 + jnp.tanh(x * (c + (c * 0.044715) * (x * x))))

def _dot(a, b):
    return jnp.dot(a, b, preferred_element_type=F32)

def _dot_nt(a, b):
    return lax.dot_general(a, b, (((1,), (1,)), ((), ())), preferred_element_type=F32)

def make(TQ=256, CH=256, PR=256):
    NQ = S // TQ
    def kernel(x_ref, wq_ref, wk_ref, wv_ref, wo_ref, w1_ref, w2_ref, w3_ref, w4_ref, o_ref,
               xn_s, k_s, vt_s, qt_s, h_s, s_s, ot_s):
        i = pl.program_id(0)

        @pl.when(i == 0)
        def _():
            wqt = wq_ref[...].T
            wvt = wv_ref[...].astype(F32).T.astype(BF16)
            h_s[0:PADR, :] = jnp.zeros((PADR, D), BF16)
            h_s[PADR + S:, :] = jnp.zeros((PADR, D), BF16)
            k_s[...] = jnp.zeros(k_s.shape, BF16)
            for c in range(S // PR):
                r = slice(c * PR, (c + 1) * PR)
                xn = _ln(x_ref[r, :].astype(F32)).astype(BF16)
                xn_s[r, :] = xn
                k_s[r, 0:DH] = _dot(xn, wk_ref[...]).astype(BF16)
                vt_s[:, r] = _dot_nt(wvt, xn).astype(BF16)
                qt = (_dot_nt(wqt, xn) * (LOG2E * DH ** -0.5)).astype(BF16)
                for j in range(PR // TQ):
                    qt_s[c * (PR // TQ) + j] = qt[:, j * TQ:(j + 1) * TQ]
                y = _ln(xn.astype(F32)).astype(BF16)
                h_s[PADR + c * PR:PADR + (c + 1) * PR, :] = _gelu(_dot(y, w1_ref[...])).astype(BF16)

        NC = S // CH
        def scores_chunk(qt, slot, c, m):
            s = _dot(k_s[c * CH:(c + 1) * CH, 0:DH], qt)
            s_s[slot, c * CH:(c + 1) * CH, :] = s
            mc = jnp.max(s.reshape(CH // 8, 8, TQ), axis=0)
            return mc if m is None else jnp.maximum(m, mc)

        def fin(m):
            return jnp.max(m, axis=0, keepdims=True)

        def pv_chunk(slot, c, m, acc, l):
            p = jnp.exp2(s_s[slot, c * CH:(c + 1) * CH, :] - m)
            lc = jnp.sum(p.reshape(CH // 8, 8, TQ), axis=0)
            a = _dot(vt_s[:, c * CH:(c + 1) * CH], p.astype(BF16))
            return (a, lc) if acc is None else (acc + a, l + lc)

        def load_q(h):
            return qt_s[i, pl.ds(pl.multiple_of(h * DH, DH), DH), :]

        def stage(h, slot, m, do_next):
            acc = l = mn = None
            if do_next:
                qn = load_q(h + 1)
            for c in range(NC):
                if do_next:
                    mn = scores_chunk(qn, 1 - slot, c, mn)
                acc, l = pv_chunk(slot, c, m, acc, l)
            o = acc / jnp.sum(l, axis=0, keepdims=True)
            ot_s[pl.ds(pl.multiple_of(h * DH, DH), DH), :] = o.astype(BF16)
            return fin(mn) if do_next else None

        m = None
        q0 = load_q(0)
        for c in range(NC):
            m = scores_chunk(q0, 0, c, m)
        m = fin(m)

        def body(t, m):
            m = stage(2 * t, 0, m, True)
            m = stage(2 * t + 1, 1, m, True)
            return m
        m = lax.fori_loop(0, H // 2 - 1, body, m)
        m = stage(H - 2, 0, m, True)
        stage(H - 1, 1, m, False)

        sa = lax.dot_general(ot_s[...], wo_ref[...], (((0,), (0,)), ((), ())), preferred_element_type=F32)
        r0 = pl.multiple_of(i * TQ, TQ)
        hh = h_s[pl.ds(r0, TQ + 2 * PADR), :].astype(F32)
        hs = jnp.concatenate([
            hh[PADR - 1:PADR - 1 + TQ, 0:128], hh[PADR + 1:PADR + 1 + TQ, 128:256],
            hh[PADR - 2:PADR - 2 + TQ, 256:384], hh[PADR + 2:PADR + 2 + TQ, 384:512]], axis=1).astype(BF16)
        x1 = xn_s[pl.ds(r0, TQ), :].astype(F32) + _dot(hs, w2_ref[...])
        y = _ln(x1).astype(BF16)
        h2 = _dot(_gelu(_dot(y, w3_ref[...])).astype(BF16), w4_ref[...])
        b = x1 + h2
        g = b * (1.0 / (1.0 + jnp.exp(-b)))
        o_ref[...] = (x_ref[pl.ds(r0, TQ), :].astype(F32) + sa * g).astype(o_ref.dtype)

    def fn(A_x, A_wq, A_wk, A_wv, A_wo, B_x, B_w1, B_w2, B_w3, B_w4):
        full = lambda a: pl.BlockSpec(a.shape, lambda i: (0, 0))
        args = (A_x.reshape(S, D), A_wq, A_wk, A_wv, A_wo, B_w1, B_w2, B_w3, B_w4)
        out = pl.pallas_call(
            kernel, grid=(NQ,),
            in_specs=[full(a) for a in args],
            out_specs=pl.BlockSpec((TQ, D), lambda i: (i, 0)),
            out_shape=jax.ShapeDtypeStruct((S, D), A_x.dtype),
            scratch_shapes=[
                pltpu.VMEM((S, D), BF16), pltpu.VMEM((S, 128), BF16), pltpu.VMEM((DH, S), BF16),
                pltpu.VMEM((NQ, D, TQ), BF16), pltpu.VMEM((S + 2 * PADR, D), BF16),
                pltpu.VMEM((2, S, TQ), F32), pltpu.VMEM((D, TQ), BF16)],
            compiler_params=pltpu.CompilerParams(dimension_semantics=("arbitrary",), vmem_limit_bytes=100 * 2**20),
            name="fused",
        )(*args)
        return out.reshape(1, S, D)
    return fn


_fn = make(TQ=512, CH=128, PR=512)


@jax.jit
def pallas_recurrent_scan__grouped_kv_mqa__mixer_s_mlp__prompt_kernel(
    A_x, A_wq, A_wk, A_wv, A_wo, B_x, B_w1, B_w2, B_w3, B_w4,
):
    return _fn(A_x, A_wq, A_wk, A_wv, A_wo, B_x, B_w1, B_w2, B_w3, B_w4)
```

```python
import jax
import jax.numpy as jnp
from jax import lax
import jax.experimental.pallas as pl
import jax.experimental.pallas.tpu as pltpu

S, D, H, DH, F = 2048, 512, 32, 16, 1792
F32, BF16 = jnp.float32, jnp.bfloat16
LOG2E = 1.4426950408889634
PADR = 16

def _ln(x):
    m = jnp.mean(x, axis=-1, keepdims=True)
    xc = x - m
    v = jnp.mean(xc * xc, axis=-1, keepdims=True)
    return xc * lax.rsqrt(v + 1e-5)

def _gelu(x):
    c = 0.7978845608028654
    return (0.5 * x) * (1.0 + jnp.tanh(x * (c + (c * 0.044715) * (x * x))))

def _dot(a, b):
    return jnp.dot(a, b, preferred_element_type=F32)

def _dot_nt(a, b):
    return lax.dot_general(a, b, (((1,), (1,)), ((), ())), preferred_element_type=F32)

def make(TQ=512, CH=128, TJ=128, PR=512, SPI=6, LAG=3, NB=3, SK=4):
    NQ = S // TQ
    NP = S // PR
    NF = F // 128
    NC = S // CH
    NJ = TQ // TJ
    NST = NQ * H

    def kernel(x_hbm, wq_hbm, wkt_hbm, wvt_hbm, wo_hbm, w1_hbm, w2_hbm, w3_hbm, w4_hbm, o_hbm,
               x_s, wq_s, wqv_s, wo_s, w1_s, w2_s, w3_s, w4_s,
               xn_s, k_s, vt_s, qt_s, h_s, s0, s1, s2, ot_s, xsem, wsem, osem):
        s_s = (s0, s1, s2)
        def rows(c, n=PR):
            return pl.ds(pl.multiple_of(c * n, n), n)
        def xcp(c):
            return pltpu.make_async_copy(x_hbm.at[rows(c)], x_s.at[rows(c)], xsem.at[c])
        def ocp(c):
            return pltpu.make_async_copy(x_s.at[rows(c)], o_hbm.at[rows(c)], osem.at[c])
        mk = pltpu.make_async_copy
        c_wq, c_wk, c_wv = mk(wq_hbm, wq_s, wsem.at[0]), mk(wkt_hbm, wqv_s.at[pl.ds(D + DH, DH)], wsem.at[1]), mk(wvt_hbm, wqv_s.at[pl.ds(D, DH)], wsem.at[2])
        c_w1, c_w2, c_wo = mk(w1_hbm, w1_s, wsem.at[3]), mk(w2_hbm, w2_s, wsem.at[4]), mk(wo_hbm, wo_s, wsem.at[5])
        c_w4 = mk(w4_hbm, w4_s, wsem.at[6])
        c_w3 = [mk(w3_hbm.at[:, pl.ds(f * 128, 128)], w3_s.at[f], wsem.at[7]) for f in range(NF)]
        for c in (c_wq, xcp(0), c_wk, c_wv, c_w1):
            c.start()
        h_s[0:PADR, :] = jnp.zeros((PADR, D), BF16)
        h_s[PADR + S:, :] = jnp.zeros((PADR, D), BF16)
        c_wq.wait()
        for c in range(1, NP):
            xcp(c).start()
        for c in [c_w2, c_wo, c_w4] + c_w3:
            c.start()
        wqv_s[0:D, :] = wq_s[...].T
        c_wk.wait()
        c_wv.wait()
        c_w1.wait()

        def pro1(c, _):
            xcp(c).wait()
            r = rows(c)
            xn = _ln(x_s[r, :].astype(F32)).astype(BF16)
            xn_s[r, :] = xn
            qv = _dot_nt(wqv_s[...], xn)
            for j in range(PR // TJ):
                cl = slice(j * TJ, (j + 1) * TJ)
                vt_s[c * (PR // TJ) + j] = qv[D:D + DH, cl].astype(BF16)
                qt_s[c * (PR // TJ) + j] = (qv[:D, cl] * (LOG2E * DH ** -0.5)).astype(BF16)
            k_s[r, :] = qv[D + DH:, :].T.astype(BF16)
            y = _ln(xn.astype(F32)).astype(BF16)
            h_s[pl.ds(pl.multiple_of(PADR + c * PR, PADR), PR), :] = _gelu(_dot(y, w1_s[...])).astype(BF16)
        lax.fori_loop(0, NP, pro1, None)
        for c in [c_w2, c_wo, c_w4] + c_w3:
            c.wait()

        def mix1(c):
            hh = h_s[pl.ds(pl.multiple_of(c * PR, PR), PR + 2 * PADR), :].astype(F32)
            hs = jnp.concatenate([
                hh[PADR - 1:PADR - 1 + PR, 0:128], hh[PADR + 1:PADR + 1 + PR, 128:256],
                hh[PADR - 2:PADR - 2 + PR, 256:384], hh[PADR + 2:PADR + 2 + PR, 384:512]], axis=1).astype(BF16)
            x1 = xn_s[rows(c), :].astype(F32) + _dot(hs, w2_s[...])
            return x1, _ln(x1).astype(BF16)

        def red8(a, op):
            return op(a.reshape(a.shape[0] // 8, 8, a.shape[1]), axis=0)
        def scores_chunk(qt, slot, c, j, m):
            s = _dot(k_s[c * CH:(c + 1) * CH, :], qt)
            s_s[slot][j, c * CH:(c + 1) * CH, :] = s
            mc = red8(s, jnp.max)
            return mc if m is None else jnp.maximum(m, mc)
        def fin(m):
            return tuple(jnp.broadcast_to(jnp.max(x, axis=0, keepdims=True), x.shape) for x in m)
        def pv_chunk(slot, c, j, m, st):
            p = jnp.exp2(s_s[slot][j, c * CH:(c + 1) * CH, :].reshape(CH // 8, 8, TJ) - m).reshape(CH, TJ)
            lc = red8(p, jnp.sum)
            a = _dot(vt_s[c], p.astype(BF16))
            return (a, lc) if st is None else (st[0] + a, st[1] + lc)
        def load_q(t):
            return [qt_s[(t // H) * NJ + j, rows(t % H, DH), :] for j in range(NJ)]
        def stages(t0, n, carry):
            m, mn = list(carry[0]), list(carry[1])
            static = isinstance(t0, int)
            hist = []
            for e in range(n):
                t = t0 + e
                st = [None] * NJ
                for c in range(NC):
                    d, g = 1 + (c + SK) // NC, (c + SK) % NC
                    live = not static or t + d < NST
                    if g == 0:
                        m_next, mn = fin(mn), [None] * NJ
                    if live and (g == 0 or c == 0):
                        qn = load_q(t + d)
                    for j in range(NJ):
                        mm = m[j]
                        if live:
                            mn[j] = scores_chunk(qn[j], (e + d) % NB, g, j, mn[j])
                            if len(hist) >= LAG:
                                mm = jnp.minimum(mm, jnp.maximum(mm, hist[-LAG][j]))
                        st[j] = pv_chunk(e % NB, c, j, mm, st[j])
                    hist.append(list(mn))
                for j in range(NJ):
                    o = st[j][0] / jnp.sum(st[j][1], axis=0, keepdims=True)
                    ot_s[(t // H) * NJ + j, rows(t % H, DH), :] = o.astype(BF16)
                m = m_next
                if mn[0] is None:
                    mn = m
            return tuple(m), tuple(mn)

        def prime(t, n):
            m = [None] * NJ
            q0 = load_q(t)
            for c in range(n):
                for j in range(NJ):
                    m[j] = scores_chunk(q0[j], t, c, j, m[j])
            return tuple(m)

        nit = (NST - 2) // SPI
        carry = (fin(prime(0, NC)), prime(1, SK))
        carry = lax.fori_loop(0, nit, lambda it, cr: stages(it * SPI, SPI, cr), carry)
        stages(nit * SPI, NST - nit * SPI, carry)

        def epi(c, _):
            r = rows(c)
            sa = jnp.concatenate([
                lax.dot_general(ot_s[c * (PR // TJ) + j], wo_s[...], (((0,), (0,)), ((), ())), preferred_element_type=F32)
                for j in range(PR // TJ)], axis=0)
            x1, y = mix1(c)
            a = jnp.concatenate([_gelu(_dot(y, w3_s[f])).astype(BF16) for f in range(NF)], axis=1)
            b = x1 + _dot(a, w4_s[...])
            g = b * (1.0 / (1.0 + jnp.exp(-b)))
            x_s[r, :] = (x_s[r, :].astype(F32) + sa * g).astype(BF16)
            ocp(c).start()
        lax.fori_loop(0, NP, epi, None)
        for c in range(NP):
            ocp(c).wait()

    def fn(A_x, A_wq, A_wk, A_wv, A_wo, B_x, B_w1, B_w2, B_w3, B_w4):
        args = (A_x.reshape(S, D), A_wq, A_wk.T, A_wv.T, A_wo, B_w1, B_w2, B_w3, B_w4)
        V = pltpu.VMEM
        out = pl.pallas_call(
            kernel,
            in_specs=[pl.BlockSpec(memory_space=pl.ANY)] * len(args),
            out_specs=pl.BlockSpec(memory_space=pl.ANY),
            out_shape=jax.ShapeDtypeStruct((S, D), A_x.dtype),
            scratch_shapes=[
                V((S, D), BF16), V((D, D), BF16), V((D + 2 * DH, D), BF16),
                V((D, D), BF16), V((D, D), BF16), V((D, D), BF16), V((NF, D, 128), BF16), V((F, D), BF16),
                V((S, D), BF16), V((S, DH), BF16), V((S // TJ, DH, TJ), BF16),
                V((S // TJ, D, TJ), BF16), V((S + 2 * PADR, D), BF16),
                V((NJ, S, TJ), F32), V((NJ, S, TJ), F32), V((NJ, S, TJ), F32), V((S // TJ, D, TJ), BF16),
                pltpu.SemaphoreType.DMA((NP,)), pltpu.SemaphoreType.DMA((8,)), pltpu.SemaphoreType.DMA((NP,))],
            compiler_params=pltpu.CompilerParams(vmem_limit_bytes=100 * 2**20),
            name="fused",
        )(*args)
        return out.reshape(1, S, D)
    return fn


_fn = make()


@jax.jit
def pallas_recurrent_scan__grouped_kv_mqa__mixer_s_mlp__prompt_kernel(
    A_x, A_wq, A_wk, A_wv, A_wo, B_x, B_w1, B_w2, B_w3, B_w4,
):
    return _fn(A_x, A_wq, A_wk, A_wv, A_wo, B_x, B_w1, B_w2, B_w3, B_w4)
```
